```python
import os as _os
_os.environ.setdefault('JAX_PLATFORMS', 'cpu')
import jax
import jax.numpy as jnp

def _softmax(x, axis=-1):
    return jax.nn.softmax(x, axis=axis)

def _gelu(x):
    return jax.nn.gelu(x, approximate=True)

def _silu(x):
    return jax.nn.silu(x)

def _sigmoid(x):
    return jax.nn.sigmoid(x)

def _layernorm(x, axis=-1, eps=1e-05):
    m = jnp.mean(x, axis=axis, keepdims=True)
    v = jnp.var(x, axis=axis, keepdims=True)
    return (x - m) / jnp.sqrt(v + eps)

def _scatter_add(tgt, idx, src, axis=0):
    return tgt.at[idx].add(src)

def _segment_sum(src, seg, n):
    return jax.ops.segment_sum(src, seg, n)

class _Rng:

    def __init__(self, key):
        self._k = key

    def _next(self):
        self._k, sub = jax.random.split(self._k)
        return sub

    def normal(self, shape):
        return jax.random.normal(self._next(), shape, dtype=jnp.bfloat16)

    def randint(self, lo, hi, shape):
        return jax.random.randint(self._next(), shape, lo, hi, dtype=jnp.int32)

    def uniform(self, shape, lo=0.0, hi=1.0):
        return jax.random.uniform(self._next(), shape, jnp.bfloat16, lo, hi)

    def permutation(self, n):
        return jax.random.permutation(self._next(), n)
kernel_name = 'adaLN_cond__ssm_conv_h3__moe_arch_mod__prompt'

def setup_inputs():
    _rng = _Rng(jax.random.key(int.from_bytes(__import__("os").urandom(4), "little")))
    _w = lambda a: (lambda t: t.astype(jnp.bfloat16) if jnp.issubdtype(t.dtype, jnp.floating) else t)(jnp.asarray(a))

    def _A_setup():
        B, S, D = (1, 2048, 640)
        ks = 4
        return {'q': _w((lambda *s: _rng.normal(s) * 0.05)(B, S, D)), 'k': _w((lambda *s: _rng.normal(s) * 0.4)(B, S, D)), 'v': _w((lambda *s: _rng.normal(s) * 0.4)(B, S, D)), 'shift_k': _w((lambda *s: _rng.normal(s) * 0.4)(D, ks) * 0.5), 'ssm_k': _w((lambda *s: _rng.normal(s) * 0.4)(D, S) * (1.0 / S ** 0.5)), 'ssm_D': _w((lambda *s: _rng.normal(s) * 0.4)(D))}
    _A_in = _A_setup()

    def _B_setup():
        B, S, D, F, C = (1, 2048, 640, 1728, 2)
        return {'x': _w((lambda *s: _rng.normal(s) * 0.05)(B, S, D)), 'w_r': _w((lambda *s: _rng.normal(s) * 0.1)(D)), 'w_gate': _w((lambda *s: _rng.normal(s) * 0.1)(D, F)), 'w_up': _w((lambda *s: _rng.normal(s) * 0.1)(D, F)), 'w_down': _w((lambda *s: _rng.normal(s) * 0.1)(F, D))}
    _B_in = _B_setup()
    return {'A_q': _A_in['q'], 'A_k': _A_in['k'], 'A_v': _A_in['v'], 'A_shift_k': _A_in['shift_k'], 'A_ssm_k': _A_in['ssm_k'], 'A_ssm_D': _A_in['ssm_D'], 'B_x': _B_in['x'], 'B_w_r': _B_in['w_r'], 'B_w_gate': _B_in['w_gate'], 'B_w_up': _B_in['w_up'], 'B_w_down': _B_in['w_down'], 'c': _w((lambda *s: _rng.normal(s) * 0.2)(1, 640) * 8.0), 'w_mod': _w((lambda *s: _rng.normal(s) * 0.2)(640, 6 * 640) * 640 ** (-0.5) * 8.0)}

def reference(A_q, A_k, A_v, A_shift_k, A_ssm_k, A_ssm_D, B_x, B_w_r, B_w_gate, B_w_up, B_w_down, c, w_mod):

    def _A_ref(q, k, v, shift_k, ssm_k, ssm_D):
        B, S, D = q.shape
        ks = shift_k.shape[-1]
        k_pad = jnp.pad(k, ((0, 0), (ks - 1, 0), (0, 0)))
        k_shift = jnp.zeros_like(k)
        for t in range(ks):
            k_shift = k_shift + k_pad[:, t:t + S, :] * shift_k[:, ks - 1 - t][None, None, :]
        kv = k_shift * v
        L = 2 * S
        kv_pad = jnp.pad(kv, ((0, 0), (0, S), (0, 0)))
        kf_pad = jnp.pad(ssm_k, ((0, 0), (0, S)))
        kv_f = (lambda x, axes=(-2, -1): jnp.fft.rfft2(x.astype(jnp.float32), axes=axes))(kv_pad[:, None, :, :], axes=(1, 2))
        kf_f = (lambda x, axes=(-2, -1): jnp.fft.rfft2(x.astype(jnp.float32), axes=axes))(kf_pad[:, None, :], axes=(1, 2))
        kf_f = (lambda x, *d: x.transpose(*d))(kf_f, 1, 2, 0)
        y_f = kv_f * kf_f[None, :, :, :]
        y = (lambda x, s, axes=(-2, -1): jnp.fft.irfft2(x, s=s, axes=axes).astype(jnp.bfloat16))(y_f, (1, L), axes=(1, 2))[:, 0, :S, :]
        y = y + kv * ssm_D[None, None, :]
        return q * y

    def _B_ref(x, w_r, w_gate, w_up, w_down):
        B, S, D = x.shape
        C = 2
        r = x @ w_r
        idx = jnp.argsort(-r, axis=-1)[:, :C]
        idx_e = jnp.repeat(idx.reshape(B, C, 1), D, axis=2)
        x_sel = jnp.take_along_axis(x, idx_e, axis=1)
        g = _silu(x_sel @ w_gate)
        u = x_sel @ w_up
        y = g * u @ w_down
        r_sel = _sigmoid(jnp.take_along_axis(r, idx, axis=1))
        y = y * r_sel.reshape(B, C, 1)
        b_off = (jnp.arange(B) * S).reshape(B, 1)
        flat_idx = (idx + b_off).reshape(B * C)
        zero = (x * 0.0).reshape(B * S, D)
        upd = _scatter_add(zero, flat_idx, y.reshape(B * C, D), axis=0)
        return x + upd.reshape(B, S, D)
    x = A_q
    mod = (_silu(c) @ w_mod).reshape(c.shape[0], 6, 1, -1)
    sa, ca, ga, sb, cb, gb = (mod[:, 0].copy(), mod[:, 1].copy(), mod[:, 2].copy(), mod[:, 3].copy(), mod[:, 4].copy(), mod[:, 5].copy())
    h = _layernorm(x, axis=-1) * (1 + ca) + sa
    x = x + ga * _A_ref(h, A_k, A_v, A_shift_k, A_ssm_k, A_ssm_D)
    h = _layernorm(x, axis=-1) * (1 + cb) + sb
    x = x + gb * _B_ref(h, B_w_r, B_w_gate, B_w_up, B_w_down)
    return x
```

```python
import math

import jax
import jax.numpy as jnp
from jax import lax
import jax.experimental.pallas as pl
import jax.experimental.pallas.tpu as pltpu

F32 = jnp.float32
BF16 = jnp.bfloat16
U32 = jnp.uint32

S = 2048
D = 640
NT = D // 128
FF = 1728
CH = 512
NCH = S // CH
NQ = 4
NO = 8
RB = 128
NB = S // RB
WD_A = 1408
SPLIT0 = 6
EPS = 1e-05

SEM_SMALL = 0
SEM_FENCE = SEM_SMALL + 4
SEM_S = SEM_FENCE + NT - 1
SEM_KV = SEM_S + NT
SEM_Q = SEM_KV + 2 * NCH
SEM_W = SEM_Q + NQ
SEM_O = SEM_W + 5
NSEM = SEM_O + NO

_NT_DIMS = (((1,), (1,)), ((), ()))


def _dot(a, b):
    return jnp.dot(a, b, preferred_element_type=F32)


def _dot_nt(a, b):
    return lax.dot_general(a, b, _NT_DIMS, preferred_element_type=F32)


def _to_u32(x):
    return pltpu.bitcast(x.astype(BF16), U32)


def _to_bf16(x):
    return pltpu.bitcast(x, BF16)


def _cmul(a, b):
    return (a[0] * b[0] - a[1] * b[1], a[0] * b[1] + a[1] * b[0])


def _lanes(c):
    return slice(128 * c, 128 * c + 128)


def _kernel(q_hbm, k_hbm, v_hbm, sw_hbm, s_hbm, d_hbm, wr_hbm, wg_hbm, wu_hbm, wd_hbm,
            c_hbm, wm_hbm, o_hbm,
            qb, kb, vb, sb, swb, db, wrb, cb, wmb, wgb, wub, wdb, ob,
            fm, gm, pm, wt, kf, kvf, tw, ox, ok0, ok1, zw0, zw1, sr, kw0, kw1,
            ya, yb, xf, x1s, st0, st1, st2, st3, xn, par, rr, fence,
            sem):
    st = [st0, st1, st2, st3]
    ok = [ok0, ok1]
    zw = [zw0, zw1]
    kw = [kw0, kw1]

    small = [
        pltpu.make_async_copy(sw_hbm, swb, sem.at[SEM_SMALL]),
        pltpu.make_async_copy(d_hbm, db, sem.at[SEM_SMALL + 1]),
        pltpu.make_async_copy(wr_hbm, wrb, sem.at[SEM_SMALL + 2]),
        pltpu.make_async_copy(c_hbm, cb, sem.at[SEM_SMALL + 3]),
    ]

    def fence_copy(u):
        return pltpu.make_async_copy(c_hbm, fence.at[u], sem.at[SEM_FENCE + u])

    def s_copy(c):
        rows = pl.ds(c * 128, 128)
        return pltpu.make_async_copy(s_hbm.at[rows], sb.at[rows], sem.at[SEM_S + c])

    def kv_copies(i):
        rows = pl.ds(i * CH, CH)
        return [
            pltpu.make_async_copy(k_hbm.at[0, rows], kb.at[rows], sem.at[SEM_KV + 2 * i]),
            pltpu.make_async_copy(v_hbm.at[0, rows], vb.at[rows], sem.at[SEM_KV + 2 * i + 1]),
        ]

    def q_copy(j):
        rows = pl.ds(j * (S // NQ), S // NQ)
        return pltpu.make_async_copy(q_hbm.at[0, rows], qb.at[rows], sem.at[SEM_Q + j])

    w_copies = [
        pltpu.make_async_copy(wm_hbm, wmb, sem.at[SEM_W]),
        pltpu.make_async_copy(wg_hbm, wgb, sem.at[SEM_W + 1]),
        pltpu.make_async_copy(wu_hbm, wub, sem.at[SEM_W + 2]),
        pltpu.make_async_copy(wd_hbm.at[pl.ds(0, WD_A)], wdb.at[pl.ds(0, WD_A)],
                              sem.at[SEM_W + 3]),
        pltpu.make_async_copy(wd_hbm.at[pl.ds(WD_A, FF - WD_A)], wdb.at[pl.ds(WD_A, FF - WD_A)],
                              sem.at[SEM_W + 4]),
    ]

    def out_copy(j):
        rows = pl.ds(j * (S // NO), S // NO)
        return pltpu.make_async_copy(ob.at[rows], o_hbm.at[0, rows], sem.at[SEM_O + j])

    for cp in small:
        cp.start()
    for u in range(NT - 1):
        fence_copy(u).start()
    s_copy(0).start()
    s_copy(1).start()
    for i in range(NCH):
        for cp in kv_copies(i):
            cp.start()
    for c in range(2, NT):
        s_copy(c).start()
    w_copies[0].start()
    for j in range(NQ):
        q_copy(j).start()
    for cp in w_copies[1:]:
        cp.start()

    wang = 2.0 * math.pi / 2048.0
    j8 = lax.broadcasted_iota(jnp.int32, (8, 128), 0)
    u8 = lax.broadcasted_iota(jnp.int32, (8, 128), 1)
    r_g = lax.broadcasted_iota(jnp.int32, (128, 128), 0)
    l_g = lax.broadcasted_iota(jnp.int32, (128, 128), 1)
    eye = jnp.where(r_g == l_g, 1.0 / 512.0, 0.0).astype(BF16)
    pm[...] = _to_u32(jnp.where(l_g == 4 * (r_g & 31) + (r_g >> 5), 1.0, 0.0))
    for p in range(4):
        ang = (((4 * u8 + p) * (4 * j8 + 1)) & 2047).astype(F32) * wang
        cur0 = (jnp.cos(ang), -jnp.sin(ang))
        rot = (jnp.broadcast_to(cur0[0][0:1], (8, 128)), jnp.broadcast_to(cur0[1][0:1], (8, 128)))
        rot = _cmul(rot, rot)
        cur1 = _cmul(cur0, rot)
        for _ in range(4):
            rot = _cmul(rot, rot)
        for b in range(8):
            fm[p, 8 * b:8 * b + 8, :] = _to_u32(jnp.concatenate(cur0, axis=0))
            fm[p, 64 + 8 * b:64 + 8 * b + 8, :] = _to_u32(jnp.concatenate(cur1, axis=0))
            if b < 7:
                cur0 = _cmul(cur0, rot)
                cur1 = _cmul(cur1, rot)
        for h in range(2):
            gm[p, h] = _to_u32(_dot_nt(eye, _to_bf16(fm[p, 64 * h:64 * h + 64, :])))

    small[0].wait()
    small[1].wait()
    swf = swb[...].astype(F32)
    dvec = db[...].astype(F32).reshape(1, D)
    for c in range(NT):
        for j in range(4):
            wt[c, 8 * j:8 * j + 8, :] = jnp.broadcast_to(swf[j:j + 1, _lanes(c)], (8, 128))
        wt[c, 32:40, :] = jnp.where(j8 == 0, dvec[:, _lanes(c)], 0.0)
    kf[:, CH:CH + 8, :] = jnp.zeros((NT, 8, 128), F32)

    def fresh(z, n):
        return z if isinstance(z, int) else lax.shift_right_logical(z, n + 2)

    def fwd_dots(ops, z):
        return [_dot(_to_bf16(fm[p + z]), ops[p]) for p in range(4)]

    def filt_regroup(c, slot):
        for j in range(S // 128):
            sr[slot, j] = sb[_lanes(c), _lanes(j)]

    def filt_transpose(slot, z):
        su = sr.bitcast(U32)
        for i in range(NCH):
            for jj in range(4):
                t = _dot_nt(_to_bf16(pm[...]), _to_bf16(su[slot + z, 4 * i + jj]))
                for p in range(4):
                    tw[slot + z, i, p, 32 * jj:32 * jj + 32, :] = t[32 * p:32 * p + 32]

    def filt_pack(c, par_, slot):
        for i in range(NCH):
            for p in range(4):
                w = tw[slot, i, p]
                if i == 0 and p == 0:
                    w = jnp.concatenate([w[0:8] + wt[c, 32:40, :], w[8:]], axis=0)
                kw[par_][i, p] = w.astype(BF16)

    def filt_forward(par_, z):
        ku = kw[par_].bitcast(U32)
        for i in range(NCH):
            o = fwd_dots([_to_bf16(ku[i + z, p]) for p in range(4)], fresh(z, i))
            for p in range(4):
                ok[par_][i, p] = o[p]

    def inverse(c, par_, z, between=None):
        zu = zw[par_].bitcast(U32)
        for i in range(NCH):
            zi = fresh(z, i)
            for p in range(4):
                rows = pl.ds(i * CH + p, 128, stride=4)
                ya[c, rows, :] = _dot(_to_bf16(gm[p + zi, 0]), _to_bf16(zu[i, p, 0:64, :]))
                yb[c, rows, :] = _dot(_to_bf16(gm[p + zi, 1]), _to_bf16(zu[i, p, 64:128, :]))
                if between is not None and p % 2 == 1:
                    between(2 * i + p // 2)

    def half_dft(load, h):
        o = [load(p) for p in range(4)]
        if h == 0:
            a = (o[0][0] + o[2][0], o[0][1] + o[2][1])
            c_ = (o[1][0] + o[3][0], o[1][1] + o[3][1])
            return [(a[0] + c_[0], a[1] + c_[1]), (a[0] - c_[0], a[1] - c_[1])]
        b_ = (o[0][0] - o[2][0], o[0][1] - o[2][1])
        d = (o[1][0] - o[3][0], o[1][1] - o[3][1])
        return [(b_[0] + d[1], b_[1] - d[0]), (b_[0] - d[1], b_[1] + d[0])]

    def spectral(c, par_, zs, b0=0, b1=16):
        okc, zwc = ok[par_], zw[par_]
        for b in range(b0, b1):
            re, im = slice(16 * b, 16 * b + 8), slice(16 * b + 8, 16 * b + 16)
            lvl1 = []
            for h in range(2):
                z = zs[h]
                kraw = [half_dft(lambda p, m=m: (okc[m + z, p, re, :], okc[m + z, p, im, :]), h)
                        for m in range(NCH)]
                kk = [kraw[0]]
                for m in range(1, NCH):
                    if b < 8:
                        kk.append([(cur[0] - prv[1], cur[1] + prv[0])
                                   for cur, prv in zip(kraw[m], kraw[m - 1])])
                    else:
                        kk.append([(cur[0] + prv[1], cur[1] - prv[0])
                                   for cur, prv in zip(kraw[m], kraw[m - 1])])
                acc = [[None, None] for _ in range(NCH)]
                for j in range(NCH):
                    xx = half_dft(
                        lambda p, j=j: (ox[c, j + z, p, re, :], ox[c, j + z, p, im, :]), h)
                    for m in range(NCH - 1 - j, -1, -1):
                        for n in range(2):
                            pr = _cmul(kk[m][n], xx[n])
                            old = acc[j + m][n]
                            acc[j + m][n] = pr if old is None else (old[0] + pr[0], old[1] + pr[1])
                lvl1.append([((y0[0] + y1[0], y0[1] + y1[1]), (y0[0] - y1[0], y0[1] - y1[1]))
                             for y0, y1 in acc])
            for i in range(NCH):
                (a, b_), (c_, d) = lvl1[0][i], lvl1[1][i]
                v = [(a[0] + c_[0], a[1] + c_[1]), (b_[0] - d[1], b_[1] + d[0]),
                     (a[0] - c_[0], a[1] - c_[1]), (b_[0] + d[1], b_[1] - d[0])]
                for p in range(4):
                    zwc[i, p, 16 * b:16 * b + 16, :] = jnp.concatenate(v[p], axis=0).astype(BF16)

    def x_chunk(i, z):
        for cp in kv_copies(i):
            cp.wait()
        base = pl.multiple_of(i * CH, CH)
        for c in range(NT):
            kf[c, 0:8, :] = kf[c, CH:CH + 8, :]
            for g in range(CH // 32):
                kf[c, 8 + 32 * g:40 + 32 * g, :] = (
                    kb[pl.ds(base + 32 * g, 32), _lanes(c)].astype(F32))
            for g in range(CH // 32):
                vv = vb[pl.ds(base + 32 * g, 32), _lanes(c)].astype(F32)
                for s in range(4):
                    r = 32 * g + 8 * s
                    acc = kf[c, 8 + r:16 + r, :] * wt[c, 0:8, :]
                    for j in range(1, 4):
                        acc = acc + kf[c, 8 + r - j:16 + r - j, :] * wt[c, 8 * j:8 * j + 8, :]
                    kvf[c, r:r + 8, :] = acc * vv[8 * s:8 * s + 8]
            o = fwd_dots([kvf[c, pl.ds(p, 128, stride=4), :].astype(BF16) for p in range(4)],
                         fresh(i, c + 1))
            for p in range(4):
                ox[c, i, p] = o[p]
        return z | lax.shift_right_logical(i, 3)

    for c in range(2):
        s_copy(c).wait()
        filt_regroup(c, 0)
        filt_transpose(0, 0)
        filt_pack(c, c, 0)
        filt_forward(c, 0)
    zo = lax.fori_loop(0, NCH, x_chunk, jnp.int32(0))
    zp = lax.shift_right_logical(zo, 1)
    s_copy(2).wait()
    filt_regroup(2, 0)
    filt_transpose(0, zo)
    spectral(0, 0, (zo, zp), 0, SPLIT0)
    s_copy(3).wait()
    s_copy(4).wait()
    for c in range(3, NT):
        filt_regroup(c, c - 2)
        filt_transpose(c - 2, zo)
    filt_pack(2, 0, zp)
    spectral(0, 0, (zo, zp), SPLIT0, 16)

    for c in range(1, NT):
        fence_copy(c - 1).wait()
        par_ = c % 2
        inverse(c - 1, 1 - par_, zo)
        if c + 1 < NT:
            filt_forward(1 - par_, zo)
        if c + 2 < NT:
            filt_pack(c + 2, par_, c)
        spectral(c, par_, (zo, zp))

    small[2].wait()
    small[3].wait()
    w_copies[0].wait()
    q_copy(0).wait()
    cf = cb[...].astype(F32)
    sc = jnp.broadcast_to(cf * jax.nn.sigmoid(cf), (8, D)).astype(BF16)
    pieces = []

    def mod_piece(n):
        if n < 6:
            pieces.append(_dot(sc, wmb[:, n * D:(n + 1) * D]))

    inverse(NT - 1, (NT - 1) % 2, zo, mod_piece)
    sa, ca, ga, sb2, cb2, gb = pieces
    wr = jnp.broadcast_to(wrb[...].astype(F32).reshape(1, D), (8, D))
    par[0] = ga * (1.0 + ca)
    par[1] = ga * sa
    par[2] = gb * (1.0 + cb2)
    par[3] = gb * sb2
    par[4] = 1.0 + cb2
    par[5] = sb2
    par[6] = gb
    wrp = (1.0 + cb2) * wr
    wr_hi = wrp.astype(BF16).astype(F32)
    row8 = lax.broadcasted_iota(jnp.int32, (8, D), 0)
    par[7] = jnp.where(row8 == 0, wr_hi, jnp.where(row8 == 1, wrp - wr_hi, 0.0))
    par[8] = jnp.broadcast_to(jnp.sum(sb2 * wr, axis=-1, keepdims=True), (8, D))

    def rowmean(tiles):
        acc = (tiles[0] + tiles[1]) + (tiles[2] + tiles[3]) + tiles[4]
        return jnp.broadcast_to(jnp.sum(acc, axis=-1, keepdims=True) * (1.0 / D), (8, 128))

    def row(base, off, mult):
        return off if base is None else pl.multiple_of(base + off, mult)

    def pass1(base, off, e):
        for s in range(RB // 8):
            rows = pl.ds(row(base, off + 8 * s, 8), 8)
            x = [qb[rows, _lanes(t)].astype(F32) for t in range(NT)]
            for t in range(NT):
                xf[t, rows, :] = x[t]
            st[0][rows, :] = rowmean(x)

    def pass2(base, off, e):
        for s in range(RB // 8):
            rows = pl.ds(row(base, off + 8 * s, 8), 8)
            m = st[0][rows, :]
            xc = [xf[t, rows, :] - m for t in range(NT)]
            st[1][rows, :] = lax.rsqrt(rowmean([a * a for a in xc]) + EPS)

    def pass3(base, off, e):
        for s in range(RB // 8):
            rows = pl.ds(row(base, off + 8 * s, 8), 8)
            m = st[0][rows, :]
            rstd = st[1][rows, :]
            x = [xf[t, rows, :] for t in range(NT)]
            x1 = [x[t] + (((x[t] - m) * rstd * par[0, :, _lanes(t)] + par[1, :, _lanes(t)])
                          * (ya[t, rows, :] + yb[t, rows, :])) for t in range(NT)]
            for t in range(NT):
                x1s[t, rows, :] = x1[t]
            st[2][rows, :] = rowmean(x1)

    def pass4(base, off, e):
        for s in range(RB // 8):
            rows = pl.ds(row(base, off + 8 * s, 8), 8)
            m = st[2][rows, :]
            xc = [x1s[t, rows, :] - m for t in range(NT)]
            st[3][rows, :] = lax.rsqrt(rowmean([a * a for a in xc]) + EPS)

    def pass5(base, off, e):
        for s in range(RB // 16):
            r0 = row(base, off + 16 * s, 16)
            m = st[2][pl.ds(r0, 16), :]
            rstd = st[3][pl.ds(r0, 16), :]
            for t in range(NT):
                x1 = x1s[t, pl.ds(r0, 16), :]
                xn2 = (x1 - m) * rstd
                xn[t, pl.ds(r0, 16), :] = xn2.astype(BF16)
                for h in range(2):
                    ob[pl.ds(r0 + 8 * h, 8), _lanes(t)] = (
                        x1[8 * h:8 * h + 8] + xn2[8 * h:8 * h + 8] * par[2, :, _lanes(t)]
                        + par[3, :, _lanes(t)]).astype(BF16)

    def pass6(base, off, e):
        r0 = pl.multiple_of(e * (RB // 2), RB // 2)
        wr8 = par[7].astype(BF16)
        acc = None
        for t in range(NT):
            part = _dot_nt(wr8[:, _lanes(t)], _to_bf16(xn.bitcast(U32)[t, pl.ds(r0, RB // 2), :]))
            acc = part if acc is None else acc + part
        rr[e] = acc

    passes = [pass1, pass2, pass3, pass4, pass5, pass6]
    npass = len(passes)
    per_q = NB // NQ

    def ep_step(e, lo, hi):
        static = isinstance(e, int)
        base = None if static else pl.multiple_of((e - (npass - 1)) * RB, RB)
        for k in (0, 1, 3, 2, 5, 4):
            if lo <= k < hi:
                passes[k](base, (e - k) * RB if static else (npass - 1 - k) * RB, e - k)

    def ep_steady(e, carry):
        @pl.when(e % per_q == 0)
        def _():
            q_copy(e // per_q).wait()
        ep_step(e, 0, npass)
        return carry

    for e in range(npass - 1):
        if e % per_q == 0 and e > 0:
            q_copy(e // per_q).wait()
        ep_step(e, 0, e + 1)
    lax.fori_loop(npass - 1, NB, ep_steady, 0)
    for e in range(NB, NB + npass - 1):
        ep_step(e, e - NB + 1, npass)

    rv = rr[:, 0, :] + rr[:, 1, :]
    pos = (lax.broadcasted_iota(jnp.int32, (NB, RB), 0) * RB
           + lax.broadcasted_iota(jnp.int32, (NB, RB), 1))
    bits = lax.bitcast_convert_type(rv, jnp.int32)
    keys = jnp.where(bits < 0, bits ^ jnp.int32(0x7FFFFFFF), bits)
    keys = (keys & jnp.int32(-S)) | (S - 1 - pos)
    k1 = jnp.max(keys, keepdims=True)
    k2 = jnp.max(jnp.where(keys == k1, jnp.int32(-2 ** 31), keys), keepdims=True)
    i1 = jnp.clip((S - 1) - (k1[0, 0] & (S - 1)), 0, S - 1)
    i2 = jnp.clip((S - 1) - (k2[0, 0] & (S - 1)), 0, S - 1)
    m1 = jnp.sum(jnp.where(keys == k1, rv, 0.0), keepdims=True)
    m2 = jnp.sum(jnp.where(keys == k2, rv, 0.0), keepdims=True)
    hit = [jnp.logical_or(i1 // (S // NO) == j, i2 // (S // NO) == j) for j in range(NO)]

    row16 = lax.broadcasted_iota(jnp.int32, (16, 128), 0)
    sel = []
    for t in range(NT):
        picked = []
        for idx in (i1, i2):
            base = pl.multiple_of((idx // 16) * 16, 16)
            blk = xn[t, pl.ds(base, 16), :].astype(F32)
            picked.append(jnp.sum(jnp.where(row16 == idx % 16, blk, 0.0), axis=0, keepdims=True))
        sel.append(jnp.where(j8 == 0, picked[0], jnp.where(j8 == 1, picked[1], 0.0)))
    hsel = (jnp.concatenate(sel, axis=1) * par[4] + par[5]).astype(BF16)

    for cp in w_copies[1:4]:
        cp.wait()
    for j in range(NO):
        @pl.when(jnp.logical_not(hit[j]))
        def _(j=j):
            out_copy(j).start()

    g = _dot_nt(hsel, wgb[...])
    u = _dot_nt(hsel, wub[...])
    act = (g * jax.nn.sigmoid(g) * u).astype(BF16)
    w_copies[4].wait()
    yf = _dot(act, wdb[...])
    r_const = par[8, 0:1, 0:1]
    gate = jnp.where(lax.broadcasted_iota(jnp.int32, (8, 1), 0) == 0,
                     jax.nn.sigmoid(m1 + r_const), jax.nn.sigmoid(m2 + r_const))
    upd = yf * gate * par[6]
    row16w = lax.broadcasted_iota(jnp.int32, (16, D), 0)
    for n, idx in enumerate((i1, i2)):
        base = pl.multiple_of((idx // 16) * 16, 16)
        blk = ob[pl.ds(base, 16), :].astype(F32)
        ob[pl.ds(base, 16), :] = (
            blk + jnp.where(row16w == idx % 16, upd[n:n + 1], 0.0)).astype(BF16)

    for j in range(NO):
        @pl.when(hit[j])
        def _(j=j):
            out_copy(j).start()
    for j in range(NO):
        out_copy(j).wait()


@jax.jit
def pallas_adaLN_cond__ssm_conv_h3__moe_arch_mod__prompt_kernel(
    A_q: jax.Array,
    A_k: jax.Array,
    A_v: jax.Array,
    A_shift_k: jax.Array,
    A_ssm_k: jax.Array,
    A_ssm_D: jax.Array,
    B_x: jax.Array,
    B_w_r: jax.Array,
    B_w_gate: jax.Array,
    B_w_up: jax.Array,
    B_w_down: jax.Array,
    c: jax.Array,
    w_mod: jax.Array,
):
    del B_x
    scratch = [
        pltpu.VMEM((S, D), BF16),
        pltpu.VMEM((S, D), BF16),
        pltpu.VMEM((S, D), BF16),
        pltpu.VMEM((D, S), BF16),
        pltpu.VMEM((4, D), BF16),
        pltpu.VMEM((D,), BF16),
        pltpu.VMEM((D,), BF16),
        pltpu.VMEM((1, D), BF16),
        pltpu.VMEM((D, 6 * D), BF16),
        pltpu.VMEM((FF, D), BF16),
        pltpu.VMEM((FF, D), BF16),
        pltpu.VMEM((FF, D), BF16),
        pltpu.VMEM((S, D), BF16),
        pltpu.VMEM((4, 128, 128), U32),
        pltpu.VMEM((4, 2, 64, 128), U32),
        pltpu.VMEM((64, 128), U32),
        pltpu.VMEM((NT, 40, 128), F32),
        pltpu.VMEM((NT, CH + 8, 128), F32),
        pltpu.VMEM((NT, CH, 128), F32),
        pltpu.VMEM((3, NCH, 4, 128, 128), F32),
        pltpu.VMEM((NT, NCH, 4, 256, 128), F32),
        pltpu.VMEM((NCH, 4, 256, 128), F32),
        pltpu.VMEM((NCH, 4, 256, 128), F32),
        pltpu.VMEM((NCH, 4, 256, 128), BF16),
        pltpu.VMEM((NCH, 4, 256, 128), BF16),
        pltpu.VMEM((3, S // 128, 128, 128), BF16),
        pltpu.VMEM((NCH, 4, 128, 128), BF16),
        pltpu.VMEM((NCH, 4, 128, 128), BF16),
        pltpu.VMEM((NT, S, 128), F32),
        pltpu.VMEM((NT, S, 128), F32),
        pltpu.VMEM((NT, S, 128), F32),
        pltpu.VMEM((NT, S, 128), F32),
        pltpu.VMEM((S, 128), F32),
        pltpu.VMEM((S, 128), F32),
        pltpu.VMEM((S, 128), F32),
        pltpu.VMEM((S, 128), F32),
        pltpu.VMEM((NT, S, 128), BF16),
        pltpu.VMEM((9, 8, D), F32),
        pltpu.VMEM((NB, 8, RB), F32),
        pltpu.VMEM((NT - 1, 1, D), BF16),
        pltpu.SemaphoreType.DMA((NSEM,)),
    ]
    any_spec = pl.BlockSpec(memory_space=pl.ANY)
    return pl.pallas_call(
        _kernel,
        in_specs=[any_spec] * 12,
        out_specs=any_spec,
        out_shape=jax.ShapeDtypeStruct(A_q.shape, A_q.dtype),
        scratch_shapes=scratch,
        compiler_params=pltpu.CompilerParams(vmem_limit_bytes=100 * 1024 * 1024),
    )(A_q, A_k, A_v, A_shift_k.T, A_ssm_k, A_ssm_D, B_w_r,
      B_w_gate.T, B_w_up.T, B_w_down, c, w_mod)
```

```python
import math

import jax
import jax.numpy as jnp
from jax import lax
import jax.experimental.pallas as pl
import jax.experimental.pallas.tpu as pltpu

F32 = jnp.float32
BF16 = jnp.bfloat16
U32 = jnp.uint32

S = 2048
D = 640
NT = D // 128
FF = 1728
CH = 512
NCH = S // CH
NQ = 4
NO = 8
RB = 128
NB = S // RB
WD_A = 1472
SPLIT0 = 6
EPS = 1e-05

SEM_SMALL = 0
SEM_FENCE = SEM_SMALL + 4
SEM_S = SEM_FENCE + NT - 1
SEM_KV = SEM_S + NT
SEM_Q = SEM_KV + 2 * NCH
SEM_W = SEM_Q + NQ
NSEM = SEM_W + 5

_NT_DIMS = (((1,), (1,)), ((), ()))


def _dot(a, b):
    return jnp.dot(a, b, preferred_element_type=F32)


def _dot_nt(a, b):
    return lax.dot_general(a, b, _NT_DIMS, preferred_element_type=F32)


def _to_u32(x):
    return pltpu.bitcast(x.astype(BF16), U32)


def _to_bf16(x):
    return pltpu.bitcast(x, BF16)


def _cmul(a, b):
    return (a[0] * b[0] - a[1] * b[1], a[0] * b[1] + a[1] * b[0])


def _lanes(c):
    return slice(128 * c, 128 * c + 128)


def _unrolled(lo, hi, body):
    def step(i, carry):
        body(i)
        return carry
    lax.fori_loop(lo, hi, step, 0, unroll=True)


def _out_copy(ob, o_hbm, osem, j):
    rows = pl.ds(j * (S // NO), S // NO)
    return pltpu.make_async_copy(ob.at[rows], o_hbm.at[0, rows], osem)


def _kernel(*refs):
    o_hbm, ob, osem = refs[12], refs[25], refs[-1]
    pl.run_scoped(lambda sem: _body(*refs, sem), pltpu.SemaphoreType.DMA((NSEM,)))
    for j in range(NO):
        _out_copy(ob, o_hbm, osem, j).wait()


def _body(q_hbm, k_hbm, v_hbm, sw_hbm, s_hbm, d_hbm, wr_hbm, wg_hbm, wu_hbm, wd_hbm,
          c_hbm, wm_hbm, o_hbm,
          qb, kb, vb, sb, swb, db, wrb, cb, wmb, wgb, wub, wdb, ob,
          fm, gm, pm, wt, kf, kvf, tw, ox, ok0, ok1, zw0, zw1, sr, kw0, kw1,
          ya, yb, xf, x1s, st0, st1, st2, st3, xn, par, rr, fence,
          osem, sem):
    st = [st0, st1, st2, st3]
    ok = [ok0, ok1]
    zw = [zw0, zw1]
    kw = [kw0, kw1]

    small = [
        pltpu.make_async_copy(sw_hbm, swb, sem.at[SEM_SMALL]),
        pltpu.make_async_copy(d_hbm, db, sem.at[SEM_SMALL + 1]),
        pltpu.make_async_copy(wr_hbm, wrb, sem.at[SEM_SMALL + 2]),
        pltpu.make_async_copy(c_hbm, cb, sem.at[SEM_SMALL + 3]),
    ]

    def fence_copy(u):
        return pltpu.make_async_copy(c_hbm, fence.at[u], sem.at[SEM_FENCE + u])

    def s_copy(c):
        rows = pl.ds(c * 128, 128)
        return pltpu.make_async_copy(s_hbm.at[rows], sb.at[rows], sem.at[SEM_S + c])

    def kv_copies(i):
        rows = pl.ds(i * CH, CH)
        return [
            pltpu.make_async_copy(k_hbm.at[0, rows], kb.at[rows], sem.at[SEM_KV + 2 * i]),
            pltpu.make_async_copy(v_hbm.at[0, rows], vb.at[rows], sem.at[SEM_KV + 2 * i + 1]),
        ]

    def q_copy(j):
        rows = pl.ds(j * (S // NQ), S // NQ)
        return pltpu.make_async_copy(q_hbm.at[0, rows], qb.at[rows], sem.at[SEM_Q + j])

    w_copies = [
        pltpu.make_async_copy(wm_hbm, wmb, sem.at[SEM_W]),
        pltpu.make_async_copy(wg_hbm, wgb, sem.at[SEM_W + 1]),
        pltpu.make_async_copy(wu_hbm, wub, sem.at[SEM_W + 2]),
        pltpu.make_async_copy(wd_hbm.at[pl.ds(0, WD_A)], wdb.at[pl.ds(0, WD_A)],
                              sem.at[SEM_W + 3]),
        pltpu.make_async_copy(wd_hbm.at[pl.ds(WD_A, FF - WD_A)], wdb.at[pl.ds(WD_A, FF - WD_A)],
                              sem.at[SEM_W + 4]),
    ]

    def out_copy(j):
        return _out_copy(ob, o_hbm, osem, j)

    for cp in small:
        cp.start()
    for u in range(NT - 1):
        fence_copy(u).start()
    s_copy(0).start()
    s_copy(1).start()
    for i in range(NCH):
        for cp in kv_copies(i):
            cp.start()
    for c in range(2, NT):
        s_copy(c).start()
    w_copies[0].start()
    for j in range(NQ):
        q_copy(j).start()
    for cp in w_copies[1:]:
        cp.start()

    wang = 2.0 * math.pi / 2048.0
    j8 = lax.broadcasted_iota(jnp.int32, (8, 128), 0)
    u8 = lax.broadcasted_iota(jnp.int32, (8, 128), 1)
    r_g = lax.broadcasted_iota(jnp.int32, (128, 128), 0)
    l_g = lax.broadcasted_iota(jnp.int32, (128, 128), 1)
    eye = jnp.where(r_g == l_g, 1.0 / 512.0, 0.0).astype(BF16)
    pm[...] = _to_u32(jnp.where(l_g == 4 * (r_g & 31) + (r_g >> 5), 1.0, 0.0))
    for p in range(4):
        ang = (((4 * u8 + p) * (4 * j8 + 1)) & 2047).astype(F32) * wang
        cur0 = (jnp.cos(ang), -jnp.sin(ang))
        rot = (jnp.broadcast_to(cur0[0][0:1], (8, 128)), jnp.broadcast_to(cur0[1][0:1], (8, 128)))
        rot = _cmul(rot, rot)
        cur1 = _cmul(cur0, rot)
        for _ in range(4):
            rot = _cmul(rot, rot)
        for b in range(8):
            fm[p, 8 * b:8 * b + 8, :] = _to_u32(jnp.concatenate(cur0, axis=0))
            fm[p, 64 + 8 * b:64 + 8 * b + 8, :] = _to_u32(jnp.concatenate(cur1, axis=0))
            if b < 7:
                cur0 = _cmul(cur0, rot)
                cur1 = _cmul(cur1, rot)
        for h in range(2):
            gm[p, h] = _to_u32(_dot_nt(eye, _to_bf16(fm[p, 64 * h:64 * h + 64, :])))

    small[0].wait()
    small[1].wait()
    swf = swb[...].astype(F32)
    dvec = db[...].astype(F32).reshape(1, D)
    for c in range(NT):
        for j in range(4):
            wt[c, 8 * j:8 * j + 8, :] = jnp.broadcast_to(swf[j:j + 1, _lanes(c)], (8, 128))
        wt[c, 32:40, :] = jnp.where(j8 == 0, dvec[:, _lanes(c)], 0.0)
    kf[:, CH:CH + 8, :] = jnp.zeros((NT, 8, 128), F32)

    def fresh(z, n):
        return z if isinstance(z, int) else lax.shift_right_logical(z, n + 2)

    def fwd_dots(ops, z):
        return [_dot(_to_bf16(fm[p + z]), ops[p]) for p in range(4)]

    def filt_regroup(c, slot):
        for j in range(S // 128):
            sr[slot, j] = sb[_lanes(c), _lanes(j)]

    def filt_transpose(slot, z):
        su = sr.bitcast(U32)
        for i in range(NCH):
            for jj in range(4):
                t = _dot_nt(_to_bf16(pm[...]), _to_bf16(su[slot + z, 4 * i + jj]))
                for p in range(4):
                    tw[slot + z, i, p, 32 * jj:32 * jj + 32, :] = t[32 * p:32 * p + 32]

    def filt_pack(c, par_, slot):
        for i in range(NCH):
            for p in range(4):
                w = tw[slot, i, p]
                if i == 0 and p == 0:
                    w = jnp.concatenate([w[0:8] + wt[c, 32:40, :], w[8:]], axis=0)
                kw[par_][i, p] = w.astype(BF16)

    def filt_forward(par_, z):
        ku = kw[par_].bitcast(U32)
        for i in range(NCH):
            o = fwd_dots([_to_bf16(ku[i + z, p]) for p in range(4)], fresh(z, i))
            for p in range(4):
                ok[par_][i, p] = o[p]

    def inverse(c, par_, z, between=None):
        zu = zw[par_].bitcast(U32)
        for i in range(NCH):
            zi = fresh(z, i)
            for p in range(4):
                rows = pl.ds(i * CH + p, 128, stride=4)
                ya[c, rows, :] = _dot(_to_bf16(gm[p + zi, 0]), _to_bf16(zu[i, p, 0:64, :]))
                yb[c, rows, :] = _dot(_to_bf16(gm[p + zi, 1]), _to_bf16(zu[i, p, 64:128, :]))
                if between is not None and p % 2 == 1:
                    between(2 * i + p // 2)

    def half_dft(load, h):
        o = [load(p) for p in range(4)]
        if h == 0:
            a = (o[0][0] + o[2][0], o[0][1] + o[2][1])
            c_ = (o[1][0] + o[3][0], o[1][1] + o[3][1])
            return [(a[0] + c_[0], a[1] + c_[1]), (a[0] - c_[0], a[1] - c_[1])]
        b_ = (o[0][0] - o[2][0], o[0][1] - o[2][1])
        d = (o[1][0] - o[3][0], o[1][1] - o[3][1])
        return [(b_[0] + d[1], b_[1] - d[0]), (b_[0] - d[1], b_[1] + d[0])]

    def spectral(c, par_, zs, b0=0, b1=16):
        okc, zwc = ok[par_], zw[par_]
        idx = [[m + z for m in range(NCH)] for z in zs]

        def slab(b, even):
            re = pl.ds(pl.multiple_of(16 * b, 16), 8)
            im = pl.ds(pl.multiple_of(16 * b + 8, 8), 8)
            lvl1 = []
            for h in range(2):
                kraw = [half_dft(lambda p, m=m: (okc[m, p, re, :], okc[m, p, im, :]), h)
                        for m in idx[h]]
                kk = [kraw[0]]
                for m in range(1, NCH):
                    if even:
                        kk.append([(cur[0] - prv[1], cur[1] + prv[0])
                                   for cur, prv in zip(kraw[m], kraw[m - 1])])
                    else:
                        kk.append([(cur[0] + prv[1], cur[1] - prv[0])
                                   for cur, prv in zip(kraw[m], kraw[m - 1])])
                acc = [[None, None] for _ in range(NCH)]
                for j in range(NCH):
                    jz = idx[h][j]
                    xx = half_dft(lambda p: (ox[c, jz, p, re, :], ox[c, jz, p, im, :]), h)
                    for m in range(NCH - 1 - j, -1, -1):
                        for n in range(2):
                            pr = _cmul(kk[m][n], xx[n])
                            old = acc[j + m][n]
                            acc[j + m][n] = pr if old is None else (old[0] + pr[0], old[1] + pr[1])
                lvl1.append([((y0[0] + y1[0], y0[1] + y1[1]), (y0[0] - y1[0], y0[1] - y1[1]))
                             for y0, y1 in acc])
            both = pl.ds(pl.multiple_of(16 * b, 16), 16)
            for i in range(NCH):
                (a, b_), (c_, d) = lvl1[0][i], lvl1[1][i]
                v = [(a[0] + c_[0], a[1] + c_[1]), (b_[0] - d[1], b_[1] + d[0]),
                     (a[0] - c_[0], a[1] - c_[1]), (b_[0] + d[1], b_[1] - d[0])]
                for p in range(4):
                    zwc[i, p, both, :] = jnp.concatenate(v[p], axis=0).astype(BF16)

        if b0 < 8:
            _unrolled(b0, min(b1, 8), lambda b: slab(b, True))
        if b1 > 8:
            _unrolled(max(b0, 8), b1, lambda b: slab(b, False))

    def x_chunk(i, z):
        for cp in kv_copies(i):
            cp.wait()
        base = pl.multiple_of(i * CH, CH)
        for c in range(NT):
            kf[c, 0:8, :] = kf[c, CH:CH + 8, :]
            taps = [wt[c, 8 * j:8 * j + 1, :] for j in range(4)]
            for r in range(0, CH, 32):
                kf[c, 8 + r:40 + r, :] = kb[pl.ds(base + r, 32), _lanes(c)].astype(F32)
            for r in range(0, CH, 32):
                acc = kf[c, 8 + r:40 + r, :] * taps[0]
                for j in range(1, 4):
                    acc = acc + kf[c, 8 + r - j:40 + r - j, :] * taps[j]
                kvf[c, r:r + 32, :] = acc * vb[pl.ds(base + r, 32), _lanes(c)].astype(F32)
            o = fwd_dots([kvf[c, pl.ds(p, 128, stride=4), :].astype(BF16) for p in range(4)],
                         fresh(i, c + 1))
            for p in range(4):
                ox[c, i, p] = o[p]
        return z | lax.shift_right_logical(i, 3)

    for c in range(2):
        s_copy(c).wait()
        filt_regroup(c, 0)
        filt_transpose(0, 0)
        filt_pack(c, c, 0)
        filt_forward(c, 0)
    zo = lax.fori_loop(0, NCH, x_chunk, jnp.int32(0))
    zp = lax.shift_right_logical(zo, 1)
    s_copy(2).wait()
    filt_regroup(2, 0)
    filt_transpose(0, zo)
    spectral(0, 0, (zo, zp), 0, SPLIT0)
    s_copy(3).wait()
    s_copy(4).wait()
    for c in range(3, NT):
        filt_regroup(c, c - 2)
        filt_transpose(c - 2, zo)
    filt_pack(2, 0, zp)
    spectral(0, 0, (zo, zp), SPLIT0, 16)

    for c in range(1, NT):
        fence_copy(c - 1).wait()
        par_ = c % 2
        inverse(c - 1, 1 - par_, zo)
        if c + 1 < NT:
            filt_forward(1 - par_, zo)
        if c + 2 < NT:
            filt_pack(c + 2, par_, c)
        spectral(c, par_, (zo, zp))

    small[2].wait()
    small[3].wait()
    w_copies[0].wait()
    q_copy(0).wait()
    cf = cb[...].astype(F32)
    sc = jnp.broadcast_to(cf * jax.nn.sigmoid(cf), (8, D)).astype(BF16)
    pieces = []

    def mod_piece(n):
        if n < 6:
            pieces.append(_dot(sc, wmb[:, n * D:(n + 1) * D]))

    inverse(NT - 1, (NT - 1) % 2, zo, mod_piece)
    sa, ca, ga, sb2, cb2, gb = pieces
    wr = jnp.broadcast_to(wrb[...].astype(F32).reshape(1, D), (8, D))
    par[0] = ga * (1.0 + ca)
    par[1] = ga * sa
    par[2] = gb * (1.0 + cb2)
    par[3] = gb * sb2
    par[4] = 1.0 + cb2
    par[5] = sb2
    par[6] = gb
    wrp = (1.0 + cb2) * wr
    wr_hi = wrp.astype(BF16).astype(F32)
    row8 = lax.broadcasted_iota(jnp.int32, (8, D), 0)
    par[7] = jnp.where(row8 == 0, wr_hi, jnp.where(row8 == 1, wrp - wr_hi, 0.0))
    par[8] = jnp.broadcast_to(jnp.sum(sb2 * wr, axis=-1, keepdims=True), (8, D))

    def rowmean(tiles):
        acc = (tiles[0] + tiles[1]) + (tiles[2] + tiles[3]) + tiles[4]
        return jnp.broadcast_to(jnp.sum(acc, axis=-1, keepdims=True) * (1.0 / D), (8, 128))

    def groups(base, off, n, body):
        start = off if base is None else base + off
        _unrolled(0, RB // n, lambda s: body(pl.multiple_of(start + n * s, n)))

    def pass1(base, off, e):
        def body(r0):
            rows = pl.ds(r0, 8)
            x = [qb[rows, _lanes(t)].astype(F32) for t in range(NT)]
            for t in range(NT):
                xf[t, rows, :] = x[t]
            st[0][rows, :] = rowmean(x)
        groups(base, off, 8, body)

    def pass2(base, off, e):
        def body(r0):
            rows = pl.ds(r0, 8)
            m = st[0][rows, :]
            xc = [xf[t, rows, :] - m for t in range(NT)]
            st[1][rows, :] = lax.rsqrt(rowmean([a * a for a in xc]) + EPS)
        groups(base, off, 8, body)

    def pass3(base, off, e):
        def body(r0):
            rows = pl.ds(r0, 8)
            m = st[0][rows, :]
            rstd = st[1][rows, :]
            x = [xf[t, rows, :] for t in range(NT)]
            x1 = [x[t] + (((x[t] - m) * rstd * par[0, :, _lanes(t)] + par[1, :, _lanes(t)])
                          * (ya[t, rows, :] + yb[t, rows, :])) for t in range(NT)]
            for t in range(NT):
                x1s[t, rows, :] = x1[t]
            st[2][rows, :] = rowmean(x1)
        groups(base, off, 8, body)

    def pass4(base, off, e):
        def body(r0):
            rows = pl.ds(r0, 8)
            m = st[2][rows, :]
            xc = [x1s[t, rows, :] - m for t in range(NT)]
            st[3][rows, :] = lax.rsqrt(rowmean([a * a for a in xc]) + EPS)
        groups(base, off, 8, body)

    def pass5(base, off, e):
        def body(r0):
            m = st[2][pl.ds(r0, 16), :]
            rstd = st[3][pl.ds(r0, 16), :]
            for t in range(NT):
                x1 = x1s[t, pl.ds(r0, 16), :]
                xn2 = (x1 - m) * rstd
                xn[t, pl.ds(r0, 16), :] = xn2.astype(BF16)
                for h in range(2):
                    ob[pl.ds(r0 + 8 * h, 8), _lanes(t)] = (
                        x1[8 * h:8 * h + 8] + xn2[8 * h:8 * h + 8] * par[2, :, _lanes(t)]
                        + par[3, :, _lanes(t)]).astype(BF16)
        groups(base, off, 16, body)

    def pass6(base, off, e):
        r0 = pl.multiple_of(e * (RB // 2), RB // 2)
        wr8 = par[7].astype(BF16)
        acc = None
        for t in range(NT):
            part = _dot_nt(wr8[:, _lanes(t)], _to_bf16(xn.bitcast(U32)[t, pl.ds(r0, RB // 2), :]))
            acc = part if acc is None else acc + part
        rr[e] = acc

    passes = [pass1, pass2, pass3, pass4, pass5, pass6]
    npass = len(passes)
    per_q = NB // NQ

    def ep_step(e, lo, hi):
        static = isinstance(e, int)
        base = None if static else pl.multiple_of((e - (npass - 1)) * RB, RB)
        for k in (0, 1, 3, 2, 5, 4):
            if lo <= k < hi:
                passes[k](base, (e - k) * RB if static else (npass - 1 - k) * RB, e - k)

    def ep_steady(e, carry):
        @pl.when(e % per_q == 0)
        def _():
            q_copy(e // per_q).wait()
        ep_step(e, 0, npass)
        return carry

    for e in range(npass - 1):
        if e % per_q == 0 and e > 0:
            q_copy(e // per_q).wait()
        ep_step(e, 0, e + 1)
    lax.fori_loop(npass - 1, NB, ep_steady, 0)
    for e in range(NB, NB + npass - 1):
        ep_step(e, e - NB + 1, npass)

    rv = rr[:, 0, :] + rr[:, 1, :]
    pos = (lax.broadcasted_iota(jnp.int32, (NB, RB), 0) * RB
           + lax.broadcasted_iota(jnp.int32, (NB, RB), 1))
    bits = lax.bitcast_convert_type(rv, jnp.int32)
    keys = jnp.where(bits < 0, bits ^ jnp.int32(0x7FFFFFFF), bits)
    keys = (keys & jnp.int32(-S)) | (S - 1 - pos)
    k1 = jnp.max(keys, keepdims=True)
    k2 = jnp.max(jnp.where(keys == k1, jnp.int32(-2 ** 31), keys), keepdims=True)
    i1 = jnp.clip((S - 1) - (k1[0, 0] & (S - 1)), 0, S - 1)
    i2 = jnp.clip((S - 1) - (k2[0, 0] & (S - 1)), 0, S - 1)
    m1 = jnp.sum(jnp.where(keys == k1, rv, 0.0), keepdims=True)
    m2 = jnp.sum(jnp.where(keys == k2, rv, 0.0), keepdims=True)
    hit = [jnp.logical_or(i1 // (S // NO) == j, i2 // (S // NO) == j) for j in range(NO)]

    row16 = lax.broadcasted_iota(jnp.int32, (16, 128), 0)
    sel = []
    for t in range(NT):
        picked = []
        for idx in (i1, i2):
            base = pl.multiple_of((idx // 16) * 16, 16)
            blk = xn[t, pl.ds(base, 16), :].astype(F32)
            picked.append(jnp.sum(jnp.where(row16 == idx % 16, blk, 0.0), axis=0, keepdims=True))
        sel.append(jnp.where(j8 == 0, picked[0], jnp.where(j8 == 1, picked[1], 0.0)))
    hsel = (jnp.concatenate(sel, axis=1) * par[4] + par[5]).astype(BF16)

    for cp in w_copies[1:4]:
        cp.wait()
    for j in range(NO):
        @pl.when(jnp.logical_not(hit[j]))
        def _(j=j):
            out_copy(j).start()

    g = _dot_nt(hsel, wgb[...])
    u = _dot_nt(hsel, wub[...])
    act = (g * jax.nn.sigmoid(g) * u).astype(BF16)
    w_copies[4].wait()
    yf = _dot(act, wdb[...])
    r_const = par[8, 0:1, 0:1]
    gate = jnp.where(lax.broadcasted_iota(jnp.int32, (8, 1), 0) == 0,
                     jax.nn.sigmoid(m1 + r_const), jax.nn.sigmoid(m2 + r_const))
    upd = yf * gate * par[6]
    row16w = lax.broadcasted_iota(jnp.int32, (16, D), 0)
    for n, idx in enumerate((i1, i2)):
        base = pl.multiple_of((idx // 16) * 16, 16)
        blk = ob[pl.ds(base, 16), :].astype(F32)
        ob[pl.ds(base, 16), :] = (
            blk + jnp.where(row16w == idx % 16, upd[n:n + 1], 0.0)).astype(BF16)

    for j in range(NO):
        @pl.when(hit[j])
        def _(j=j):
            out_copy(j).start()


@jax.jit
def pallas_adaLN_cond__ssm_conv_h3__moe_arch_mod__prompt_kernel(
    A_q: jax.Array,
    A_k: jax.Array,
    A_v: jax.Array,
    A_shift_k: jax.Array,
    A_ssm_k: jax.Array,
    A_ssm_D: jax.Array,
    B_x: jax.Array,
    B_w_r: jax.Array,
    B_w_gate: jax.Array,
    B_w_up: jax.Array,
    B_w_down: jax.Array,
    c: jax.Array,
    w_mod: jax.Array,
):
    del B_x
    scratch = [
        pltpu.VMEM((S, D), BF16),
        pltpu.VMEM((S, D), BF16),
        pltpu.VMEM((S, D), BF16),
        pltpu.VMEM((D, S), BF16),
        pltpu.VMEM((4, D), BF16),
        pltpu.VMEM((D,), BF16),
        pltpu.VMEM((D,), BF16),
        pltpu.VMEM((1, D), BF16),
        pltpu.VMEM((D, 6 * D), BF16),
        pltpu.VMEM((FF, D), BF16),
        pltpu.VMEM((FF, D), BF16),
        pltpu.VMEM((FF, D), BF16),
        pltpu.VMEM((S, D), BF16),
        pltpu.VMEM((4, 128, 128), U32),
        pltpu.VMEM((4, 2, 64, 128), U32),
        pltpu.VMEM((64, 128), U32),
        pltpu.VMEM((NT, 40, 128), F32),
        pltpu.VMEM((NT, CH + 8, 128), F32),
        pltpu.VMEM((NT, CH, 128), F32),
        pltpu.VMEM((3, NCH, 4, 128, 128), F32),
        pltpu.VMEM((NT, NCH, 4, 256, 128), F32),
        pltpu.VMEM((NCH, 4, 256, 128), F32),
        pltpu.VMEM((NCH, 4, 256, 128), F32),
        pltpu.VMEM((NCH, 4, 256, 128), BF16),
        pltpu.VMEM((NCH, 4, 256, 128), BF16),
        pltpu.VMEM((3, S // 128, 128, 128), BF16),
        pltpu.VMEM((NCH, 4, 128, 128), BF16),
        pltpu.VMEM((NCH, 4, 128, 128), BF16),
        pltpu.VMEM((NT, S, 128), F32),
        pltpu.VMEM((NT, S, 128), F32),
        pltpu.VMEM((NT, S, 128), F32),
        pltpu.VMEM((NT, S, 128), F32),
        pltpu.VMEM((S, 128), F32),
        pltpu.VMEM((S, 128), F32),
        pltpu.VMEM((S, 128), F32),
        pltpu.VMEM((S, 128), F32),
        pltpu.VMEM((NT, S, 128), BF16),
        pltpu.VMEM((9, 8, D), F32),
        pltpu.VMEM((NB, 8, RB), F32),
        pltpu.VMEM((NT - 1, 1, D), BF16),
        pltpu.SemaphoreType.DMA,
    ]
    any_spec = pl.BlockSpec(memory_space=pl.ANY)
    return pl.pallas_call(
        _kernel,
        in_specs=[any_spec] * 12,
        out_specs=any_spec,
        out_shape=jax.ShapeDtypeStruct(A_q.shape, A_q.dtype),
        scratch_shapes=scratch,
        compiler_params=pltpu.CompilerParams(vmem_limit_bytes=100 * 1024 * 1024),
    )(A_q, A_k, A_v, A_shift_k.T, A_ssm_k, A_ssm_D, B_w_r,
      B_w_gate.T, B_w_up.T, B_w_down, c, w_mod)
```
